```python
import jax
import jax.numpy as jnp

def _softmax(x, axis=-1):
    return jax.nn.softmax(x, axis=axis)
def _gelu(x):
    return jax.nn.gelu(x, approximate=True)
def _silu(x):
    return jax.nn.silu(x)
def _sigmoid(x):
    return jax.nn.sigmoid(x)
def _layernorm(x, axis=-1, eps=1e-5):
    m = jnp.mean(x, axis=axis, keepdims=True)
    v = jnp.var(x, axis=axis, keepdims=True)
    return (x - m) / jnp.sqrt(v + eps)
def _scatter_add(tgt, idx, src, axis=0):
    return tgt.at[idx].add(src)
def _segment_sum(src, seg, n):
    return jax.ops.segment_sum(src, seg, n)
class _Rng:
    def __init__(self, key):
        self._k = key
    def _next(self):
        self._k, sub = jax.random.split(self._k)
        return sub
    def normal(self, shape):
        return jax.random.normal(self._next(), shape, dtype=jnp.bfloat16)
    def randint(self, lo, hi, shape):
        return jax.random.randint(self._next(), shape, lo, hi, dtype=jnp.int32)
    def uniform(self, shape, lo=0.0, hi=1.0):
        return jax.random.uniform(self._next(), shape, jnp.bfloat16, lo, hi)
    def permutation(self, n):
        return jax.random.permutation(self._next(), n)


kernel_name = 'standalone__depthwise_separable__vision'

def setup_inputs():
    _rng = _Rng(jax.random.key(int.from_bytes(__import__("os").urandom(4), "little")))
    _w = (lambda a: (lambda t: t.astype(jnp.bfloat16) if jnp.issubdtype(t.dtype, jnp.floating) else t)(jnp.asarray(a)))
    H = W = 384
    C = 384
    k = 1
    return {
        "x": _w((lambda *s: _rng.normal(s) * 0.05)(1, H, W, C)),
        "dw": _w((lambda *s: _rng.normal(s) * 0.05)(k, k, C)),
        "pw": _w((lambda *s: _rng.normal(s) * 0.05)(C, C)),
    }

def reference(x, dw, pw):
    B, H, W, C = x.shape
    k = dw.shape[0]
    pad = k // 2
    xp = jnp.pad(x, ((0,0),(pad,pad),(pad,pad),(0,0)))
    out = jnp.zeros_like(x)
    for i in range(k):
        for j in range(k):
            out = out + xp[:, i:i+H, j:j+W, :] * dw[i, j][None, None, None, :]
    return jnp.einsum('bhwc,cd->bhwd', out, pw)
```

```python
import jax
import jax.experimental.pallas as pl
import jax.experimental.pallas.tpu as pltpu
import jax.numpy as jnp
from jax import lax

BM = 1024

RG = 8
RH = 8
RCH = 32
PRE_GROUPS = 2
READ_RATE = 2
SWITCH = 65
TAIL_ROWS = 128

WG = 6
WCH = 32
WPRE = 64
WPS = 8


def _div(a, n):
    return lax.shift_right_logical(a, jnp.int32(n.bit_length() - 1))


def _mod(a, n):
    return a & (n - 1)


def _kernel(x_hbm, dw_hbm, pw_hbm, o_hbm, buf, dw_ref, pw_ref, rsem, wsem, csem):
    nb = buf.shape[0]
    n_rgroups = nb // RG
    sub = RG // RH
    q_group = BM // RCH
    q_step = q_group * READ_RATE // RG
    q_pre = PRE_GROUPS * q_group
    g_read = (n_rgroups - PRE_GROUPS) // READ_RATE
    w_group = BM // WCH
    n_writes = (nb // WG) * w_group

    assert q_pre + g_read * RG * q_step == n_rgroups * q_group
    assert g_read * RG <= SWITCH <= (n_rgroups - 1) * RG
    assert WPRE <= (SWITCH // WG) * w_group
    assert all(
        WPRE + (s + 1) * WPS <= ((SWITCH + s) // WG) * w_group
        for s in range(nb - SWITCH)
    )

    def start_read(q):
        g = _div(q, q_group)
        r = pl.multiple_of(_mod(q, q_group) * RCH, RCH)
        sem = g + jnp.where((g == n_rgroups - 1) & (r >= BM - TAIL_ROWS), 1, 0)
        for h in range(RH):
            blocks = pl.ds(g * RG + h * sub, sub)
            pltpu.make_async_copy(
                x_hbm.at[blocks, pl.ds(r, RCH)],
                buf.at[blocks, pl.ds(r, RCH)],
                rsem.at[sem],
            ).start(priority=h % 2)

    def wait_reads(g, sem, r0=0, rows=BM):
        blocks = pl.ds(g * RG, RG)
        pltpu.make_async_copy(
            x_hbm.at[blocks, pl.ds(r0, rows)],
            buf.at[blocks, pl.ds(r0, rows)],
            rsem.at[sem],
        ).wait()

    def start_write(k):
        blocks = pl.ds(_div(k, w_group) * WG, WG)
        r = pl.multiple_of(_mod(k, w_group) * WCH, WCH)
        pltpu.make_async_copy(
            buf.at[blocks, pl.ds(r, WCH)],
            o_hbm.at[blocks, pl.ds(r, WCH)],
            wsem.at[0],
        ).start()

    def compute(b):
        scaled = buf[b].astype(jnp.float32) * dw_ref[...].astype(jnp.float32)
        acc = jnp.dot(
            scaled.astype(buf.dtype), pw_ref[...], preferred_element_type=jnp.float32
        )
        buf[b] = acc.astype(buf.dtype)

    lax.fori_loop(0, q_group, lambda q, _: start_read(q), None)
    dw_copy = pltpu.make_async_copy(dw_hbm, dw_ref, csem.at[0])
    pw_copy = pltpu.make_async_copy(pw_hbm, pw_ref, csem.at[1])
    dw_copy.start()
    pw_copy.start()
    lax.fori_loop(q_group, q_pre, lambda q, _: start_read(q), None)
    dw_copy.wait()
    pw_copy.wait()

    def read_and_compute_group(g, _):
        wait_reads(g, g)

        def step(j, _):
            b = g * RG + j
            for u in range(q_step):
                start_read(q_pre + b * q_step + u)
            compute(b)

        lax.fori_loop(0, RG, step, None)

    lax.fori_loop(0, g_read, read_and_compute_group, None)

    def compute_while_reads_drain(b, _):
        @pl.when(_mod(b, RG) == 0)
        def _():
            wait_reads(_div(b, RG), _div(b, RG))

        compute(b)

    lax.fori_loop(g_read * RG, SWITCH, compute_while_reads_drain, None)

    last = n_rgroups - 1
    lax.fori_loop(pl.cdiv(SWITCH, RG), last, lambda g, _: wait_reads(g, g), None)
    wait_reads(last, last, 0, BM - TAIL_ROWS)
    lax.fori_loop(0, WPRE, lambda k, _: start_write(k), None)
    wait_reads(last, last + 1, BM - TAIL_ROWS, TAIL_ROWS)

    def write_and_compute(s, _):
        for u in range(WPS):
            start_write(WPRE + s * WPS + u)
        compute(SWITCH + s)

    lax.fori_loop(0, nb - SWITCH, write_and_compute, None)
    lax.fori_loop(
        WPRE + (nb - SWITCH) * WPS, n_writes, lambda k, _: start_write(k), None
    )
    pltpu.make_async_copy(buf, o_hbm, wsem.at[0]).wait()


@jax.jit
def pallas_standalone__depthwise_separable__vision_kernel(
    x: jax.Array,
    dw: jax.Array,
    pw: jax.Array,
):
    B, H, W, C = x.shape
    assert dw.shape == (1, 1, C) and pw.shape == (C, C)
    nb = B * H * W // BM
    assert nb * BM == B * H * W and nb % RG == 0 and nb % WG == 0

    out = pl.pallas_call(
        _kernel,
        in_specs=[pl.BlockSpec(memory_space=pl.ANY)] * 3,
        out_specs=pl.BlockSpec(memory_space=pl.ANY),
        out_shape=jax.ShapeDtypeStruct((nb, BM, C), x.dtype),
        scratch_shapes=[
            pltpu.VMEM((nb, BM, C), x.dtype),
            pltpu.VMEM((1, C), dw.dtype),
            pltpu.VMEM((C, C), pw.dtype),
            pltpu.SemaphoreType.DMA((nb // RG + 1,)),
            pltpu.SemaphoreType.DMA((1,)),
            pltpu.SemaphoreType.DMA((2,)),
        ],
        compiler_params=pltpu.CompilerParams(
            vmem_limit_bytes=124 * 2**20, disable_bounds_checks=True
        ),
    )(x.reshape(nb, BM, C), dw.reshape(1, C), pw)
    return out.reshape(B, H, W, C)
```

```python
import jax
import jax.experimental.pallas as pl
import jax.experimental.pallas.tpu as pltpu
import jax.numpy as jnp
from jax import lax

BM = 1024
CH = 32
CHUNKS = BM // CH

RG = 12
R_PRE = 44
R_STEP = 5
R_TAIL = 3
WG = 6
W_PRE = 12
W_STEP = 9


def _kernel(x_hbm, dw_hbm, pw_hbm, o_hbm, buf, dw_ref, pw_ref, rsem, wsem, csem):
    nb = buf.shape[0]
    half = nb // 2
    last = nb // RG - 1
    n_reads = (nb // RG) * CHUNKS
    n_writes = (nb // WG) * CHUNKS
    switch = (n_reads - R_PRE) // R_STEP

    assert half % RG == 0 and half % WG == 0
    assert R_PRE >= CHUNKS and R_PRE + switch * R_STEP == n_reads
    assert switch <= last * RG
    assert all(
        R_PRE + g * RG * R_STEP >= (g + 1) * CHUNKS
        for g in range(pl.cdiv(switch, RG))
    )
    assert W_PRE <= (switch // WG) * CHUNKS
    assert all(
        W_PRE + (s + 1) * W_STEP <= ((switch + s) // WG) * CHUNKS
        for s in range(nb - switch)
    )

    def sweep(i, group_size):
        g = lax.shift_right_logical(i, jnp.int32(CHUNKS.bit_length() - 1))
        row = pl.multiple_of((i & (CHUNKS - 1)) * CH, CH)
        block = g * group_size
        lower = jnp.where(block >= half, 1, 0)
        return g, block, row, block - lower * half, pl.multiple_of(lower * BM + row, CH)

    def start_reads(i):
        g, block, row, seg, hbm_row = sweep(i, RG)
        sem = rsem.at[g + jnp.where(i >= n_reads - R_TAIL, 1, 0)]
        for j in range(RG):
            pltpu.make_async_copy(
                x_hbm.at[seg + j, pl.ds(hbm_row, CH)],
                buf.at[block + j, pl.ds(row, CH)],
                sem,
            ).start(priority=j % 2)

    def wait_reads(g, sem, row=0, rows=BM):
        region = buf.at[pl.ds(g * RG, RG), pl.ds(row, rows)]
        pltpu.make_async_copy(region, region, rsem.at[sem]).wait()

    def start_writes(i):
        _, block, row, seg, hbm_row = sweep(i, WG)
        for j in range(WG):
            pltpu.make_async_copy(
                buf.at[block + j, pl.ds(row, CH)],
                o_hbm.at[seg + j, pl.ds(hbm_row, CH)],
                wsem.at[0],
            ).start(priority=j % 2)

    def conv(x):
        depthwise = x.astype(jnp.float32) * dw_ref[...].astype(jnp.float32)
        acc = jnp.dot(
            depthwise.astype(x.dtype), pw_ref[...], preferred_element_type=jnp.float32
        )
        return acc.astype(x.dtype)

    lax.fori_loop(0, CHUNKS, lambda i, _: start_reads(i), None)
    dw_copy = pltpu.make_async_copy(dw_hbm, dw_ref, csem.at[0])
    pw_copy = pltpu.make_async_copy(pw_hbm, pw_ref, csem.at[1])
    dw_copy.start()
    pw_copy.start()
    lax.fori_loop(CHUNKS, R_PRE, lambda i, _: start_reads(i), None)
    dw_copy.wait()
    pw_copy.wait()

    def read_step(b, _):
        @pl.when(b % RG == 0)
        def _():
            wait_reads(b // RG, b // RG)

        x = buf[b]
        for u in range(R_STEP):
            start_reads(R_PRE + b * R_STEP + u)
        buf[b] = conv(x)

    lax.fori_loop(0, switch, read_step, None)

    split = BM - R_TAIL * CH
    lax.fori_loop(pl.cdiv(switch, RG), last, lambda g, _: wait_reads(g, g), None)
    wait_reads(last, last, 0, split)
    lax.fori_loop(0, W_PRE, lambda i, _: start_writes(i), None)
    wait_reads(last, last + 1, split, BM - split)

    def write_step(s, _):
        for u in range(W_STEP):
            start_writes(W_PRE + s * W_STEP + u)
        buf[switch + s] = conv(buf[switch + s])

    lax.fori_loop(0, nb - switch, write_step, None)
    lax.fori_loop(
        W_PRE + (nb - switch) * W_STEP, n_writes, lambda i, _: start_writes(i), None
    )
    pltpu.make_async_copy(buf, buf, wsem.at[0]).wait()


@jax.jit
def pallas_standalone__depthwise_separable__vision_kernel(
    x: jax.Array,
    dw: jax.Array,
    pw: jax.Array,
):
    B, H, W, C = x.shape
    assert dw.shape == (1, 1, C) and pw.shape == (C, C)
    nb = B * H * W // BM
    assert nb * BM == B * H * W and nb % 2 == 0
    hbm_shape = (nb // 2, 2 * BM, C)

    out = pl.pallas_call(
        _kernel,
        in_specs=[pl.BlockSpec(memory_space=pl.ANY)] * 3,
        out_specs=pl.BlockSpec(memory_space=pl.ANY),
        out_shape=jax.ShapeDtypeStruct(hbm_shape, x.dtype),
        scratch_shapes=[
            pltpu.VMEM((nb, BM, C), x.dtype),
            pltpu.VMEM((1, C), dw.dtype),
            pltpu.VMEM((C, C), pw.dtype),
            pltpu.SemaphoreType.DMA((nb // RG + 1,)),
            pltpu.SemaphoreType.DMA((1,)),
            pltpu.SemaphoreType.DMA((2,)),
        ],
        compiler_params=pltpu.CompilerParams(
            vmem_limit_bytes=124 * 2**20, disable_bounds_checks=True
        ),
    )(x.reshape(hbm_shape), dw.reshape(1, C), pw)
    return out.reshape(B, H, W, C)
```
